```python
import os as _os
_os.environ.setdefault("JAX_PLATFORMS", "cpu")
import jax
import jax.numpy as jnp

def _softmax(x, axis=-1):
    return jax.nn.softmax(x, axis=axis)
def _gelu(x):
    return jax.nn.gelu(x, approximate=True)
def _silu(x):
    return jax.nn.silu(x)
def _sigmoid(x):
    return jax.nn.sigmoid(x)
def _layernorm(x, axis=-1, eps=1e-5):
    m = jnp.mean(x, axis=axis, keepdims=True)
    v = jnp.var(x, axis=axis, keepdims=True)
    return (x - m) / jnp.sqrt(v + eps)
def _scatter_add(tgt, idx, src, axis=0):
    return tgt.at[idx].add(src)
def _segment_sum(src, seg, n):
    return jax.ops.segment_sum(src, seg, n)
class _Rng:
    def __init__(self, key):
        self._k = key
    def _next(self):
        self._k, sub = jax.random.split(self._k)
        return sub
    def normal(self, shape):
        return jax.random.normal(self._next(), shape, dtype=jnp.bfloat16)
    def randint(self, lo, hi, shape):
        return jax.random.randint(self._next(), shape, lo, hi, dtype=jnp.int32)
    def uniform(self, shape, lo=0.0, hi=1.0):
        return jax.random.uniform(self._next(), shape, jnp.bfloat16, lo, hi)
    def permutation(self, n):
        return jax.random.permutation(self._next(), n)


kernel_name = 'standalone__gqa_block_cached__sampling'

def setup_inputs():
    _rng = _Rng(jax.random.key(int.from_bytes(__import__("os").urandom(4), "little")))
    _w = (lambda a: (lambda t: t.astype(jnp.bfloat16) if jnp.issubdtype(t.dtype, jnp.floating) else t)(jnp.asarray(a)))
    B, Sq, D = 32, 16, 1024
    Hq, Hkv, Sk, Dh = 32, 4, 2048, 128
    assert Hq % Hkv == 0, (Hq, Hkv)
    return {
        "x": _w((lambda *s: _rng.normal(s) * 0.8)(B, Sq, D)),
        "k_cache": _w((lambda *s: _rng.normal(s) * 0.8)(B, Hkv, Sk, Dh)),
        "v_cache": _w((lambda *s: _rng.normal(s) * 0.05)(B, Hkv, Sk, Dh)),
        "wq": _w((lambda *s: _rng.normal(s) * 0.8)(D, Hq * Dh) * (D ** -0.5)),
        "wo": _w((lambda *s: _rng.normal(s) * 0.05)(Hq * Dh, D) * ((Hq * Dh) ** -0.5)),
    }

def reference(x, k_cache, v_cache, wq, wo):
    B, Sq, D = x.shape
    Hq, Dh = 32, 128
    Hkv = k_cache.shape[1]
    rep = Hq // Hkv
    q = (lambda x, *d: x.transpose(*d))((x @ wq).reshape(B, Sq, Hq, Dh), 0, 2, 1, 3)
    k = jnp.repeat(k_cache, rep, axis=1)
    v = jnp.repeat(v_cache, rep, axis=1)
    scores = jnp.einsum("bhqd,bhkd->bhqk", q, k) * (Dh ** -0.5)
    p = _softmax(scores, axis=-1)
    o = jnp.einsum("bhqk,bhkd->bhqd", p, v)
    return (lambda x, *d: x.transpose(*d))(o, 0, 2, 1, 3).reshape(B, Sq, Hq * Dh) @ wo
```

```python
import functools
import math

import jax
import jax.numpy as jnp
from jax import lax
from jax.experimental import pallas as pl
from jax.experimental.pallas import tpu as pltpu

_NBUF = 6
_ROWS = 128


def _gqa_kernel(x_hbm, k_hbm, v_hbm, wq_hbm, wo_hbm, out_hbm,
                x_v, wq_v, wo_v, kbuf, vbuf, q_s, o_s, out_s,
                ksem, vsem, wsem, osem,
                *, B, SQ, HQ, HKV, DH, NBUF, CB):
    REP = HQ // HKV
    scale = float(DH) ** -0.5
    rows = CB * SQ

    def k_copy(b, slot):
        return pltpu.make_async_copy(k_hbm.at[b], kbuf.at[slot], ksem.at[slot])

    def v_copy(b, slot):
        return pltpu.make_async_copy(v_hbm.at[b], vbuf.at[slot], vsem.at[slot])

    x_cp = pltpu.make_async_copy(x_hbm, x_v, wsem.at[0])
    wq_cp = pltpu.make_async_copy(wq_hbm, wq_v, wsem.at[1])
    wo_cp = pltpu.make_async_copy(wo_hbm, wo_v, wsem.at[2])

    def out_copy(c):
        return pltpu.make_async_copy(out_s.at[pl.ds(c * rows, rows)],
                                     out_hbm.at[pl.ds(c * rows, rows)],
                                     osem.at[c])

    x_cp.start()
    wq_cp.start()
    for b in range(NBUF):
        k_copy(b, b).start()
        v_copy(b, b).start()
    wo_cp.start()
    x_cp.wait()
    wq_cp.wait()

    def body(b, carry):
        c = b // CB
        bl = b % CB
        slot = b % NBUF

        @pl.when(bl == 0)
        def _():
            r0 = pl.multiple_of(c * rows, rows)
            xq = x_v[pl.ds(r0, rows), :]
            q_s[...] = jnp.dot(xq, wq_v[...],
                               preferred_element_type=jnp.float32
                               ).astype(q_s.dtype)

        k_copy(b, slot).wait()
        v_copy(b, slot).wait()

        row0 = pl.multiple_of(bl * SQ, SQ)
        for g in range(HKV):
            q = jnp.concatenate(
                [q_s[pl.ds(row0, SQ), (g * REP + j) * DH:(g * REP + j + 1) * DH]
                 for j in range(REP)], axis=0)
            s = lax.dot_general(q, kbuf[slot, g], (((1,), (1,)), ((), ())),
                                preferred_element_type=jnp.float32)
            m = jnp.max(s, axis=1, keepdims=True)
            p = jnp.exp((s - m) * scale)
            l = jnp.sum(p, axis=1, keepdims=True)
            o = jnp.dot(p.astype(vbuf.dtype), vbuf[slot, g],
                        preferred_element_type=jnp.float32)
            o = (o * (1.0 / l)).astype(o_s.dtype)
            for j in range(REP):
                o_s[pl.ds(row0, SQ), (g * REP + j) * DH:(g * REP + j + 1) * DH] = (
                    o[j * SQ:(j + 1) * SQ, :])

        @pl.when(b + NBUF < B)
        def _():
            k_copy(b + NBUF, slot).start()
            v_copy(b + NBUF, slot).start()

        @pl.when(b == CB - 1)
        def _():
            wo_cp.wait()

        @pl.when(bl == CB - 1)
        def _():
            r0 = pl.multiple_of(c * rows, rows)
            out_s[pl.ds(r0, rows), :] = jnp.dot(
                o_s[...], wo_v[...], preferred_element_type=jnp.float32
            ).astype(out_s.dtype)
            out_copy(c).start()

        return carry

    lax.fori_loop(0, B, body, 0)

    for c in range(B // CB):
        out_copy(c).wait()


@jax.jit
def pallas_standalone__gqa_block_cached__sampling_kernel(
    x: jax.Array,
    k_cache: jax.Array,
    v_cache: jax.Array,
    wq: jax.Array,
    wo: jax.Array,
):
    B, SQ, D = x.shape
    _, HKV, SK, DH = k_cache.shape
    HQ = wq.shape[1] // DH
    CB = _ROWS // SQ
    assert B % CB == 0 and HQ % HKV == 0
    nbuf = min(_NBUF, B)
    x2 = x.reshape(B * SQ, D)
    dt = x.dtype

    kern = functools.partial(_gqa_kernel, B=B, SQ=SQ, HQ=HQ, HKV=HKV, DH=DH,
                             NBUF=nbuf, CB=CB)
    out = pl.pallas_call(
        kern,
        out_shape=jax.ShapeDtypeStruct((B * SQ, D), dt),
        in_specs=[pl.BlockSpec(memory_space=pl.ANY)] * 5,
        out_specs=pl.BlockSpec(memory_space=pl.ANY),
        scratch_shapes=[
            pltpu.VMEM((B * SQ, D), dt),
            pltpu.VMEM(wq.shape, dt),
            pltpu.VMEM(wo.shape, dt),
            pltpu.VMEM((nbuf, HKV, SK, DH), dt),
            pltpu.VMEM((nbuf, HKV, SK, DH), dt),
            pltpu.VMEM((CB * SQ, HQ * DH), dt),
            pltpu.VMEM((CB * SQ, HQ * DH), dt),
            pltpu.VMEM((B * SQ, D), dt),
            pltpu.SemaphoreType.DMA((nbuf,)),
            pltpu.SemaphoreType.DMA((nbuf,)),
            pltpu.SemaphoreType.DMA((3,)),
            pltpu.SemaphoreType.DMA((B // CB,)),
        ],
        compiler_params=pltpu.CompilerParams(
            vmem_limit_bytes=100 * 1024 * 1024),
    )(x2, k_cache, v_cache, wq, wo)
    return out.reshape(B, SQ, D)
```

```python
import functools

import jax
import jax.numpy as jnp
from jax import lax
from jax.experimental import pallas as pl
from jax.experimental.pallas import tpu as pltpu

_ROWS = 128
_LOG2E = 1.4426950408889634


def _gqa_kernel(x_hbm, k_hbm, v_hbm, wq_hbm, wo_hbm, out_hbm,
                x_v, wq_v, wo_v, kbuf, vbuf, q_s, o_s, acc_s, out_s,
                ksem, vsem, wsem, osem,
                *, B, SQ, HQ, HKV, DH, CB):
    REP = HQ // HKV
    GW = REP * DH
    c_exp = (float(DH) ** -0.5) * _LOG2E
    rows = CB * SQ
    n_stages = (B // CB) * HKV

    def k_copy(s, bl):
        return pltpu.make_async_copy(
            k_hbm.at[(s // HKV) * CB + bl, s % HKV], kbuf.at[bl], ksem.at[bl])

    def v_copy(s, bl):
        return pltpu.make_async_copy(
            v_hbm.at[(s // HKV) * CB + bl, s % HKV], vbuf.at[bl], vsem.at[bl])

    x_cp = pltpu.make_async_copy(x_hbm, x_v, wsem.at[0])
    wq_cp = pltpu.make_async_copy(wq_hbm, wq_v, wsem.at[1])
    wo_cp = pltpu.make_async_copy(wo_hbm, wo_v, wsem.at[2])

    def out_copy(c):
        return pltpu.make_async_copy(out_s.at[pl.ds(c * rows, rows)],
                                     out_hbm.at[pl.ds(c * rows, rows)],
                                     osem.at[c])

    x_cp.start()
    wq_cp.start()
    x_cp.wait()
    wq_cp.wait()
    for bl in range(CB):
        k_copy(0, bl).start()
        v_copy(0, bl).start()
    wo_cp.start()

    def stage(s, prefetch):
        c = s // HKV
        g = s % HKV
        r0 = pl.multiple_of(c * rows, rows)
        col0 = pl.multiple_of(g * GW, GW)

        q_s[...] = jnp.dot(x_v[pl.ds(r0, rows), :], wq_v[:, pl.ds(col0, GW)],
                           preferred_element_type=jnp.float32).astype(q_s.dtype)

        for bl in range(CB):
            k_copy(s, bl).wait()
            v_copy(s, bl).wait()
            q = jnp.concatenate(
                [q_s[bl * SQ:(bl + 1) * SQ, j * DH:(j + 1) * DH]
                 for j in range(REP)], axis=0)
            sc = lax.dot_general(q, kbuf[bl], (((1,), (1,)), ((), ())),
                                 preferred_element_type=jnp.float32)
            m = jnp.max(sc, axis=1, keepdims=True)
            p = jnp.exp2((sc - m) * c_exp)
            l = jnp.sum(p, axis=1, keepdims=True)
            o = jnp.dot(p.astype(vbuf.dtype), vbuf[bl],
                        preferred_element_type=jnp.float32)
            o = (o * (1.0 / l)).astype(o_s.dtype)
            for j in range(REP):
                o_s[bl * SQ:(bl + 1) * SQ, j * DH:(j + 1) * DH] = (
                    o[j * SQ:(j + 1) * SQ, :])
            if prefetch:
                k_copy(s + 1, bl).start()
                v_copy(s + 1, bl).start()

        @pl.when(s == 0)
        def _():
            wo_cp.wait()

        part = jnp.dot(o_s[...], wo_v[pl.ds(col0, GW), :],
                       preferred_element_type=jnp.float32)

        @pl.when(g == 0)
        def _():
            acc_s[...] = part

        @pl.when(jnp.logical_and(g > 0, g < HKV - 1))
        def _():
            acc_s[...] += part

        @pl.when(g == HKV - 1)
        def _():
            out_s[pl.ds(r0, rows), :] = (acc_s[...] + part).astype(out_s.dtype)
            out_copy(c).start()

    def loop_body(s, carry):
        stage(s, True)
        return carry

    lax.fori_loop(0, n_stages - 1, loop_body, 0)
    stage(n_stages - 1, False)

    for c in range(B // CB):
        out_copy(c).wait()


@jax.jit
def pallas_standalone__gqa_block_cached__sampling_kernel(
    x: jax.Array,
    k_cache: jax.Array,
    v_cache: jax.Array,
    wq: jax.Array,
    wo: jax.Array,
):
    B, SQ, D = x.shape
    _, HKV, SK, DH = k_cache.shape
    HQ = wq.shape[1] // DH
    CB = _ROWS // SQ
    assert B % CB == 0 and HQ % HKV == 0 and HKV >= 2
    x2 = x.reshape(B * SQ, D)
    dt = x.dtype
    gw = (HQ // HKV) * DH

    kern = functools.partial(_gqa_kernel, B=B, SQ=SQ, HQ=HQ, HKV=HKV, DH=DH,
                             CB=CB)
    out = pl.pallas_call(
        kern,
        out_shape=jax.ShapeDtypeStruct((B * SQ, D), dt),
        in_specs=[pl.BlockSpec(memory_space=pl.ANY)] * 5,
        out_specs=pl.BlockSpec(memory_space=pl.ANY),
        scratch_shapes=[
            pltpu.VMEM((B * SQ, D), dt),
            pltpu.VMEM(wq.shape, dt),
            pltpu.VMEM(wo.shape, dt),
            pltpu.VMEM((CB, SK, DH), dt),
            pltpu.VMEM((CB, SK, DH), dt),
            pltpu.VMEM((CB * SQ, gw), dt),
            pltpu.VMEM((CB * SQ, gw), dt),
            pltpu.VMEM((CB * SQ, D), jnp.float32),
            pltpu.VMEM((B * SQ, D), dt),
            pltpu.SemaphoreType.DMA((CB,)),
            pltpu.SemaphoreType.DMA((CB,)),
            pltpu.SemaphoreType.DMA((3,)),
            pltpu.SemaphoreType.DMA((B // CB,)),
        ],
        compiler_params=pltpu.CompilerParams(
            vmem_limit_bytes=100 * 1024 * 1024),
    )(x2, k_cache, v_cache, wq, wo)
    return out.reshape(B, SQ, D)
```
